```python
import os as _os
_os.environ.setdefault("JAX_PLATFORMS", "cpu")
import jax
import jax.numpy as jnp

def _softmax(x, axis=-1):
    return jax.nn.softmax(x, axis=axis)
def _gelu(x):
    return jax.nn.gelu(x, approximate=True)
def _silu(x):
    return jax.nn.silu(x)
def _sigmoid(x):
    return jax.nn.sigmoid(x)
def _layernorm(x, axis=-1, eps=1e-5):
    m = jnp.mean(x, axis=axis, keepdims=True)
    v = jnp.var(x, axis=axis, keepdims=True)
    return (x - m) / jnp.sqrt(v + eps)
def _scatter_add(tgt, idx, src, axis=0):
    return tgt.at[idx].add(src)
def _segment_sum(src, seg, n):
    return jax.ops.segment_sum(src, seg, n)
class _Rng:
    def __init__(self, key):
        self._k = key
    def _next(self):
        self._k, sub = jax.random.split(self._k)
        return sub
    def normal(self, shape):
        return jax.random.normal(self._next(), shape, dtype=jnp.bfloat16)
    def randint(self, lo, hi, shape):
        return jax.random.randint(self._next(), shape, lo, hi, dtype=jnp.int32)
    def uniform(self, shape, lo=0.0, hi=1.0):
        return jax.random.uniform(self._next(), shape, jnp.bfloat16, lo, hi)
    def permutation(self, n):
        return jax.random.permutation(self._next(), n)


kernel_name = 'concat_heads__mha_block_cached__mha_block_cached__near_ridge'

def setup_inputs():
    _rng = _Rng(jax.random.key(int.from_bytes(__import__("os").urandom(4), "little")))
    _w = (lambda a: (lambda t: t.astype(jnp.bfloat16) if jnp.issubdtype(t.dtype, jnp.floating) else t)(jnp.asarray(a)))
    def _A_setup():
        B, Sq, D = 32, 32, 640
        H, Sk, Dh = 32, 32, 128
        return {
            "x": _w((lambda *s: _rng.normal(s) * 0.8)(B, Sq, D)),
            "k_cache": _w((lambda *s: _rng.normal(s) * 0.8)(B, H, Sk, Dh)),
            "v_cache": _w((lambda *s: _rng.normal(s) * 0.05)(B, H, Sk, Dh)),
            "wq": _w((lambda *s: _rng.normal(s) * 0.8)(D, H * Dh) * (D ** -0.5)),
            "wo": _w((lambda *s: _rng.normal(s) * 0.05)(H * Dh, D) * ((H * Dh) ** -0.5)),
        }
    _A_in = _A_setup()

    def _B_setup():
        B, Sq, D = 32, 32, 640
        H, Sk, Dh = 32, 32, 128
        return {
            "x": _w((lambda *s: _rng.normal(s) * 0.8)(B, Sq, D)),
            "k_cache": _w((lambda *s: _rng.normal(s) * 0.8)(B, H, Sk, Dh)),
            "v_cache": _w((lambda *s: _rng.normal(s) * 0.05)(B, H, Sk, Dh)),
            "wq": _w((lambda *s: _rng.normal(s) * 0.8)(D, H * Dh) * (D ** -0.5)),
            "wo": _w((lambda *s: _rng.normal(s) * 0.05)(H * Dh, D) * ((H * Dh) ** -0.5)),
        }
    _B_in = _B_setup()

    return {
        "A_x": _A_in["x"],
        "A_k_cache": _A_in["k_cache"],
        "A_v_cache": _A_in["v_cache"],
        "A_wq": _A_in["wq"],
        "A_wo": _A_in["wo"],
        "B_x": _B_in["x"],
        "B_k_cache": _B_in["k_cache"],
        "B_v_cache": _B_in["v_cache"],
        "B_wq": _B_in["wq"],
        "B_wo": _B_in["wo"],
    }

def reference(A_x, A_k_cache, A_v_cache, A_wq, A_wo, B_x, B_k_cache, B_v_cache, B_wq, B_wo):
    def _A_ref(x, k_cache, v_cache, wq, wo):
        B, Sq, D = x.shape
        H, Dh = 32, 128
        q = (lambda x, *d: x.transpose(*d))((x @ wq).reshape(B, Sq, H, Dh), 0, 2, 1, 3)
        scores = jnp.einsum("bhqd,bhkd->bhqk", q, k_cache) * (Dh ** -0.5)
        p = _softmax(scores, axis=-1)
        o = jnp.einsum("bhqk,bhkd->bhqd", p, v_cache)
        return (lambda x, *d: x.transpose(*d))(o, 0, 2, 1, 3).reshape(B, Sq, H * Dh) @ wo

    def _B_ref(x, k_cache, v_cache, wq, wo):
        B, Sq, D = x.shape
        H, Dh = 32, 128
        q = (lambda x, *d: x.transpose(*d))((x @ wq).reshape(B, Sq, H, Dh), 0, 2, 1, 3)
        scores = jnp.einsum("bhqd,bhkd->bhqk", q, k_cache) * (Dh ** -0.5)
        p = _softmax(scores, axis=-1)
        o = jnp.einsum("bhqk,bhkd->bhqd", p, v_cache)
        return (lambda x, *d: x.transpose(*d))(o, 0, 2, 1, 3).reshape(B, Sq, H * Dh) @ wo

    a = _A_ref(A_x, A_k_cache, A_v_cache, A_wq, A_wo)
    b = _B_ref(B_x, B_k_cache, B_v_cache, B_wq, B_wo)
    return jnp.concatenate([a, b], axis=-1)
```

```python
import functools, os
import jax
import jax.numpy as jnp
from jax import lax
from jax.experimental import pallas as pl
from jax.experimental.pallas import tpu as pltpu

B, SQ, D = 32, 32, 640
H, SK, DH = 32, 32, 128
HG = 4
NG = H // HG
NS = 2 * NG
M = B * SQ
HW = HG * DH
SCALE = float(jnp.asarray(DH ** -0.5, jnp.bfloat16))
CB = int(os.environ.get('CB', '8'))
NC = B // CB
CR = CB * SQ
QC = int(os.environ.get('QC', '4'))
QR = M // QC
ORDER_LAST = os.environ.get('ORDER_LAST', 'S0 S1 S2 S3 P0 P1 O0 P2 O1 P3 O2 O3')
ORDER = os.environ.get('ORDER', 'S0 Q0 P0 S1 Q1 P1 S2 O0 P2 S3 O1 P3 Q2 O2 O3 Q3')


XP = os.environ.get('XP', '1') == '1'


def att_s(b, q_scr, k_ref, p_scr, lane):
    r0 = b * SQ
    qs = jnp.concatenate(
        [q_scr[r0:r0 + SQ, h * DH:(h + 1) * DH] for h in range(HG)], axis=0)
    ks = k_ref[b].reshape(HG * SK, DH)
    st = lax.dot_general(ks, qs, (((1,), (1,)), ((), ())),
                         preferred_element_type=jnp.float32)
    c = st[0:SK]
    for h in range(1, HG):
        c = jnp.where(lane == h, st[h * SK:(h + 1) * SK], c)
    m = jnp.max(c, axis=0, keepdims=True)
    e = jnp.exp((c - m) * SCALE)
    l = jnp.sum(e, axis=0, keepdims=True)
    p = e * pl.reciprocal(l, approx=False)
    ptd = jnp.concatenate([jnp.where(lane == h, p, 0.0) for h in range(HG)], axis=0).astype(jnp.bfloat16)
    if XP:
        p_scr[b] = ptd.T
    else:
        p_scr[b] = ptd


def att_pv(b, p_scr, v_ref, o_scr):
    r0 = b * SQ
    vs = v_ref[b].reshape(HG * SK, DH)
    if XP:
        o = jnp.dot(p_scr[b], vs, preferred_element_type=jnp.float32).astype(jnp.bfloat16)
    else:
        o = lax.dot_general(p_scr[b], vs, (((0,), (0,)), ((), ())),
                            preferred_element_type=jnp.float32).astype(jnp.bfloat16)
    for h in range(HG):
        o_scr[r0:r0 + SQ, h * DH:(h + 1) * DH] = o[h * SQ:(h + 1) * SQ]


def _kernel(xa, ka, va, wqa, woa, xb, kb, vb, wqb, wob, out_hbm,
            x_buf, k_buf, v_buf, wq_buf, wo_buf, acc_ref, q0, q1, o_scr, p_scr, out_buf,
            x_sem, wq_sem, kv_sem, out_sem):
    s = pl.program_id(0)
    slot = s % 2

    def wq_copy(wq_hbm, gg, sl):
        return pltpu.make_async_copy(
            wq_hbm.at[:, pl.ds(pl.multiple_of(gg * HW, HW), HW)], wq_buf.at[sl], wq_sem.at[sl])

    def kvo_copies(refs, gg, sl):
        k_hbm, v_hbm, wo_hbm = refs
        return [
            pltpu.make_async_copy(k_hbm.at[:, pl.ds(gg * HG, HG)], k_buf.at[sl], kv_sem.at[sl, 0]),
            pltpu.make_async_copy(v_hbm.at[:, pl.ds(gg * HG, HG)], v_buf.at[sl], kv_sem.at[sl, 1]),
            pltpu.make_async_copy(wo_hbm.at[pl.ds(pl.multiple_of(gg * HW, HW), HW), :], wo_buf.at[sl], kv_sem.at[sl, 2]),
        ]

    def start_wq(ss):
        gg = ss % NG
        sl = ss % 2

        @pl.when(ss < NG)
        def _():
            wq_copy(wqa, gg, sl).start()

        @pl.when(ss >= NG)
        def _():
            wq_copy(wqb, gg, sl).start()

    def start_kvo(ss):
        gg = ss % NG
        sl = ss % 2

        @pl.when(ss < NG)
        def _():
            for c in kvo_copies((ka, va, woa), gg, sl):
                c.start()

        @pl.when(ss >= NG)
        def _():
            for c in kvo_copies((kb, vb, wob), gg, sl):
                c.start()

    def qproj(x_ref, wq_ref, q_out):
        for c in range(QC):
            r = c * QR
            q = jnp.dot(x_ref[r:r + QR, :], wq_ref[...], preferred_element_type=jnp.float32)
            q_out[r:r + QR, :] = q.astype(jnp.bfloat16)

    @pl.when(s == 0)
    def _():
        xc = pltpu.make_async_copy(xa, x_buf.at[0], x_sem.at[0])
        xc.start()
        wq_copy(wqa, 0, 0).start()
        acc_ref[...] = jnp.zeros_like(acc_ref)
        xc.wait()
        wq_copy(wqa, 0, 0).wait()
        start_kvo(0)
        start_wq(1)
        qproj(x_buf.at[0], wq_buf.at[0], q0)

    @pl.when(jnp.logical_and(s > 0, s + 1 < NS))
    def _():
        start_kvo(s + 1)

    @pl.when(jnp.logical_and(s > 0, s + 2 < NS))
    def _():
        start_wq(s + 2)

    @pl.when(s == 1)
    def _():
        pltpu.make_async_copy(xb, x_buf.at[1], x_sem.at[1]).start()

    for c in kvo_copies((ka, va, woa), 0, slot):
        c.wait()

    @pl.when(s + 1 < NS)
    def _():
        wq_copy(wqa, 0, 1 - slot).wait()

    @pl.when(s == NG - 1)
    def _():
        pltpu.make_async_copy(xb, x_buf.at[1], x_sem.at[1]).wait()

    @pl.when(s == 0)
    def _():
        start_kvo(1)
        start_wq(2)

    k_ref = k_buf.at[slot]
    v_ref = v_buf.at[slot]
    wo_ref = wo_buf.at[slot]

    def body(q_cur, q_next):
        lane = lax.broadcasted_iota(jnp.int32, (SK, HG * SQ), 1) // SQ

        def sph(c):
            for b in range(c * CB, (c + 1) * CB):
                att_s(b, q_cur, k_ref, p_scr, lane)

        def pvph(c):
            for b in range(c * CB, (c + 1) * CB):
                att_pv(b, p_scr, v_ref, o_scr)

        def oproj(c):
            r = c * CR
            acc_ref[r:r + CR, :] += jnp.dot(o_scr[r:r + CR, :], wo_ref[...],
                                            preferred_element_type=jnp.float32)

        def qchunk(c):
            r = c * QR
            x_ref = x_buf.at[(s + 1) // NG]
            q = jnp.dot(x_ref[r:r + QR, :], wq_buf[1 - slot], preferred_element_type=jnp.float32)
            q_next[r:r + QR, :] = q.astype(jnp.bfloat16)

        for tok in (ORDER if q_next is not None else ORDER_LAST).split():
            kind, idx = tok[0], int(tok[1:])
            if kind == 'S':
                sph(idx)
            elif kind == 'P':
                pvph(idx)
            elif kind == 'O':
                oproj(idx)
            elif kind == 'Q' and q_next is not None:
                qchunk(idx)

    @pl.when(slot == 0)
    def _():
        body(q0, q1)

    @pl.when(jnp.logical_and(slot == 1, s < NS - 1))
    def _():
        body(q1, q0)

    @pl.when(s == NS - 1)
    def _():
        body(q1, None)

    def out_copy(blk):
        return pltpu.make_async_copy(out_buf.at[blk], out_hbm.at[:, pl.ds(blk * D, D)], out_sem.at[blk])

    @pl.when(s == NG - 1)
    def _():
        out_buf[0] = acc_ref[...].astype(out_buf.dtype)
        out_copy(0).start()
        acc_ref[...] = jnp.zeros_like(acc_ref)

    @pl.when(s == NS - 1)
    def _():
        out_buf[1] = acc_ref[...].astype(out_buf.dtype)
        out_copy(1).start()
        out_copy(0).wait()
        out_copy(1).wait()


@jax.jit
def pallas_concat_heads__mha_block_cached__mha_block_cached__near_ridge_kernel(
    A_x, A_k_cache, A_v_cache, A_wq, A_wo, B_x, B_k_cache, B_v_cache, B_wq, B_wo):
    xa = A_x.reshape(M, D)
    xb = B_x.reshape(M, D)
    bf = jnp.bfloat16
    out = pl.pallas_call(
        _kernel,
        grid=(NS,),
        in_specs=[pl.BlockSpec(memory_space=pl.ANY)] * 10,
        out_specs=pl.BlockSpec(memory_space=pl.ANY),
        out_shape=jax.ShapeDtypeStruct((M, 2 * D), bf),
        scratch_shapes=[
            pltpu.VMEM((2, M, D), bf),
            pltpu.VMEM((2, B, HG, SK, DH), bf),
            pltpu.VMEM((2, B, HG, SK, DH), bf),
            pltpu.VMEM((2, D, HW), bf),
            pltpu.VMEM((2, HW, D), bf),
            pltpu.VMEM((M, D), jnp.float32),
            pltpu.VMEM((M, HW), bf),
            pltpu.VMEM((M, HW), bf),
            pltpu.VMEM((M, HW), bf),
            pltpu.VMEM((B, HG * SK, HG * SQ), bf),
            pltpu.VMEM((2, M, D), bf),
            pltpu.SemaphoreType.DMA((2,)),
            pltpu.SemaphoreType.DMA((2,)),
            pltpu.SemaphoreType.DMA((2, 3)),
            pltpu.SemaphoreType.DMA((2,)),
        ],
        compiler_params=pltpu.CompilerParams(
            dimension_semantics=("arbitrary",),
            vmem_limit_bytes=64 * 1024 * 1024,
        ),
    )(xa, A_k_cache, A_v_cache, A_wq, A_wo, xb, B_k_cache, B_v_cache, B_wq, B_wo)
    return out.reshape(B, SQ, 2 * D)
```

```python
import jax
import jax.numpy as jnp
from jax import lax
from jax.experimental import pallas as pl
from jax.experimental.pallas import tpu as pltpu

B, SQ, D = 32, 32, 640
H, SK, DH = 32, 32, 128
HG = 4
NG = H // HG
NS = 2 * NG
M = B * SQ
HW = HG * DH
SCALE = float(jnp.asarray(DH ** -0.5, jnp.bfloat16))
CB = 8
NC = B // CB
CR = CB * SQ
NSTEP = 10
NSL = 4
XSPLIT = (0, 512, M)

ORDER = 'S0 Q0 P0 S1 O0 P1 S2 Q1 P2 S3 O1 P3 Q2 O2 Q3 O3'
ORDER_COPY = 'S0 S1 S2 S3 P0 P1 O0 C0 P2 O1 C1 P3 O2 C2 O3 C3'
ORDER_LAST = 'S0 S1 S2 S3 P0 P1 O0 P2 O1 P3 O2 O3'


def _att_scores(b, q_scr, k_ref, p_scr, lane):
    r0 = b * SQ
    qs = jnp.concatenate(
        [q_scr[r0:r0 + SQ, h * DH:(h + 1) * DH] for h in range(HG)], axis=0)
    ks = k_ref[b].reshape(HG * SK, DH)
    st = lax.dot_general(ks, qs, (((1,), (1,)), ((), ())),
                         preferred_element_type=jnp.float32)
    c = st[0:SK]
    for h in range(1, HG):
        c = jnp.where(lane == h, st[h * SK:(h + 1) * SK], c)
    m = jnp.max(c, axis=0, keepdims=True)
    e = jnp.exp((c - m) * SCALE)
    l = jnp.sum(e, axis=0, keepdims=True)
    p = e * pl.reciprocal(l, approx=False)
    ptd = jnp.concatenate(
        [jnp.where(lane == h, p, 0.0) for h in range(HG)],
        axis=0).astype(jnp.bfloat16)
    p_scr[b] = ptd.T


def _att_pv(b, p_scr, v_ref, o_scr):
    r0 = b * SQ
    vs = v_ref[b].reshape(HG * SK, DH)
    o = jnp.dot(p_scr[b], vs,
                preferred_element_type=jnp.float32).astype(jnp.bfloat16)
    for h in range(HG):
        o_scr[r0:r0 + SQ, h * DH:(h + 1) * DH] = o[h * SQ:(h + 1) * SQ]


def _kernel(xa, ka, va, wqa, woa, xb, kb, vb, wqb, wob, out_hbm,
            x_buf, k_buf, v_buf, wq_buf, wo_buf, acc_ref, q_scr, q_tmp, o_scr,
            p_scr, out_buf, x_sem, wq_sem, kv_sem, out_sem):
    st = pl.program_id(0)

    def wq_copy(wq_hbm, gg, sl):
        return pltpu.make_async_copy(
            wq_hbm.at[:, pl.ds(pl.multiple_of(gg * HW, HW), HW)],
            wq_buf.at[sl], wq_sem.at[sl])

    def kvo_copies(refs, gg, sl):
        k_hbm, v_hbm, wo_hbm = refs
        return [
            pltpu.make_async_copy(k_hbm.at[:, pl.ds(gg * HG, HG)],
                                  k_buf.at[sl], kv_sem.at[sl, 0]),
            pltpu.make_async_copy(v_hbm.at[:, pl.ds(gg * HG, HG)],
                                  v_buf.at[sl], kv_sem.at[sl, 1]),
            pltpu.make_async_copy(
                wo_hbm.at[pl.ds(pl.multiple_of(gg * HW, HW), HW), :],
                wo_buf.at[sl], kv_sem.at[sl, 2]),
        ]

    def start_wq(ss):
        gg = ss % NG
        sl = ss % NSL

        @pl.when(ss < NG)
        def _():
            wq_copy(wqa, gg, sl).start()

        @pl.when(jnp.logical_and(ss >= NG, ss < NS))
        def _():
            wq_copy(wqb, gg, sl).start()

    def start_kvo(ss):
        gg = ss % NG
        sl = ss % NSL

        @pl.when(ss < NG)
        def _():
            for c in kvo_copies((ka, va, woa), gg, sl):
                c.start()

        @pl.when(jnp.logical_and(ss >= NG, ss < NS))
        def _():
            for c in kvo_copies((kb, vb, wob), gg, sl):
                c.start()

    def wait_kvo(ss):
        for c in kvo_copies((ka, va, woa), 0, ss % NSL):
            c.wait()

    def wait_wq(ss):
        wq_copy(wqa, 0, ss % NSL).wait()

    def xb_copy():
        return pltpu.make_async_copy(xb, x_buf.at[1], x_sem.at[0])

    def out_copy(blk, c=None):
        if c is None:
            return pltpu.make_async_copy(
                out_buf.at[blk], out_hbm.at[:, pl.ds(blk * D, D)],
                out_sem.at[0])
        return pltpu.make_async_copy(
            out_buf.at[blk, pl.ds(c * CR, CR)],
            out_hbm.at[pl.ds(c * CR, CR), pl.ds(blk * D, D)],
            out_sem.at[1 + c])

    def group(gi, last=False, copy_q=False):
        k_ref = k_buf.at[gi % NSL]
        v_ref = v_buf.at[gi % NSL]
        wo_ref = wo_buf.at[gi % NSL]
        lane = lax.broadcasted_iota(jnp.int32, (SK, HG * SQ), 1) // SQ
        not_first = (gi % NG) != 0
        o_ref = out_buf.at[gi // NG]

        def sph(c):
            for b in range(c * CB, (c + 1) * CB):
                _att_scores(b, q_scr, k_ref, p_scr, lane)

        def pvph(c):
            for b in range(c * CB, (c + 1) * CB):
                _att_pv(b, p_scr, v_ref, o_scr)

        def oproj(c):
            r = c * CR
            upd = jnp.dot(o_scr[r:r + CR, :], wo_ref[...],
                          preferred_element_type=jnp.float32)
            if isinstance(not_first, bool):
                new = acc_ref[r:r + CR, :] + upd if not_first else upd
            else:
                new = jnp.where(not_first, acc_ref[r:r + CR, :], 0.0) + upd
            if not last:
                acc_ref[r:r + CR, :] = new
            o_ref[r:r + CR, :] = new.astype(out_buf.dtype)
            if last:
                out_copy(1, c).start()

        def qchunk(c):
            r = c * CR
            x_ref = x_buf.at[(gi + 1) // NG]
            q = jnp.dot(x_ref[r:r + CR, :], wq_buf[(gi + 1) % NSL],
                        preferred_element_type=jnp.float32)
            q_scr[r:r + CR, :] = q.astype(jnp.bfloat16)

        order = ORDER_LAST if last else (ORDER_COPY if copy_q else ORDER)
        for tok in order.split():
            kind, idx = tok[0], int(tok[1:])
            if kind == 'S':
                sph(idx)
            elif kind == 'P':
                pvph(idx)
            elif kind == 'O':
                oproj(idx)
            elif kind == 'Q':
                qchunk(idx)
            else:
                q_scr[idx * CR:(idx + 1) * CR, :] = (
                    q_tmp[idx * CR:(idx + 1) * CR, :])

    @pl.when(st == 0)
    def _():
        nx = len(XSPLIT) - 1

        def xc(c):
            lo, sz = XSPLIT[c], XSPLIT[c + 1] - XSPLIT[c]
            return pltpu.make_async_copy(
                xa.at[pl.ds(lo, sz)], x_buf.at[0, pl.ds(lo, sz)],
                x_sem.at[1 + c])

        wq_copy(wqa, 0, 0).start()
        xc(0).start()
        wq_copy(wqa, 0, 0).wait()
        for xi in range(nx):
            xc(xi).wait()
            if xi == 0:
                for c in range(1, nx):
                    xc(c).start()
                start_wq(1)
            if xi == nx - 1:
                start_kvo(0)
            for r in range(XSPLIT[xi], XSPLIT[xi + 1], CR):
                q = jnp.dot(x_buf[0, r:r + CR, :], wq_buf[0],
                            preferred_element_type=jnp.float32)
                q_scr[r:r + CR, :] = q.astype(jnp.bfloat16)
        wait_wq(1)
        start_kvo(1)
        start_wq(2)
        for c in range(NC):
            r = c * CR
            q = jnp.dot(x_buf[0, r:r + CR, :], wq_buf[1],
                        preferred_element_type=jnp.float32)
            q_tmp[r:r + CR, :] = q.astype(jnp.bfloat16)
        wait_kvo(0)
        start_kvo(2)
        start_wq(3)
        start_kvo(3)
        start_wq(4)
        group(0, copy_q=True)

    @pl.when(jnp.logical_or(st == 1, st == NSTEP - 2))
    def _():
        gi = jnp.where(st == 1, 1, NS - 2)
        wait_kvo(gi)
        wait_wq(gi + 1)
        group(gi)

    @pl.when(jnp.logical_and(st >= 2, st < NSTEP - 2))
    def _():
        g1 = 2 * st - 2

        @pl.when(st == NG // 2)
        def _():
            xb_copy().wait()

        wait_kvo(g1)
        wait_wq(g1 + 1)
        wait_kvo(g1 + 1)
        wait_wq(g1 + 2)
        start_kvo(g1 + 2)
        start_wq(g1 + 3)
        start_kvo(g1 + 3)
        start_wq(g1 + 4)

        @pl.when(st == 2)
        def _():
            xb_copy().start()

        group(g1)
        group(g1 + 1)

        @pl.when(st == NG // 2)
        def _():
            out_copy(0).start()

    @pl.when(st == NSTEP - 1)
    def _():
        wait_kvo(NS - 1)
        group(NS - 1, last=True)
        out_copy(0).wait()
        for c in range(NC):
            out_copy(1, c).wait()


@jax.jit
def pallas_concat_heads__mha_block_cached__mha_block_cached__near_ridge_kernel(
    A_x: jax.Array,
    A_k_cache: jax.Array,
    A_v_cache: jax.Array,
    A_wq: jax.Array,
    A_wo: jax.Array,
    B_x: jax.Array,
    B_k_cache: jax.Array,
    B_v_cache: jax.Array,
    B_wq: jax.Array,
    B_wo: jax.Array,
):
    xa = A_x.reshape(M, D)
    xb = B_x.reshape(M, D)
    bf = jnp.bfloat16
    out = pl.pallas_call(
        _kernel,
        grid=(NSTEP,),
        in_specs=[pl.BlockSpec(memory_space=pl.ANY)] * 10,
        out_specs=pl.BlockSpec(memory_space=pl.ANY),
        out_shape=jax.ShapeDtypeStruct((M, 2 * D), bf),
        scratch_shapes=[
            pltpu.VMEM((2, M, D), bf),
            pltpu.VMEM((NSL, B, HG, SK, DH), bf),
            pltpu.VMEM((NSL, B, HG, SK, DH), bf),
            pltpu.VMEM((NSL, D, HW), bf),
            pltpu.VMEM((NSL, HW, D), bf),
            pltpu.VMEM((M, D), jnp.float32),
            pltpu.VMEM((M, HW), bf),
            pltpu.VMEM((M, HW), bf),
            pltpu.VMEM((M, HW), bf),
            pltpu.VMEM((B, HG * SK, HG * SQ), bf),
            pltpu.VMEM((2, M, D), bf),
            pltpu.SemaphoreType.DMA((len(XSPLIT),)),
            pltpu.SemaphoreType.DMA((NSL,)),
            pltpu.SemaphoreType.DMA((NSL, 3)),
            pltpu.SemaphoreType.DMA((1 + NC,)),
        ],
        compiler_params=pltpu.CompilerParams(
            dimension_semantics=("arbitrary",),
            vmem_limit_bytes=64 * 1024 * 1024,
            disable_bounds_checks=True,
        ),
    )(xa, A_k_cache, A_v_cache, A_wq, A_wo,
      xb, B_k_cache, B_v_cache, B_wq, B_wo)
    return out.reshape(B, SQ, 2 * D)
```

```python
import jax
import jax.numpy as jnp
from jax import lax
from jax.experimental import pallas as pl
from jax.experimental.pallas import tpu as pltpu

B, SQ, D = 32, 32, 640
H, SK, DH = 32, 32, 128
HG = 4
NG = H // HG
NS = 2 * NG
M = B * SQ
HW = HG * DH
SCALE = 0.08837890625
CB = 8
NC = B // CB
CR = CB * SQ
NSTEP = 10
NSL = 4
XR = M // 2

ORDER = 'S0 Q0 P0 S1 O0 P1 S2 Q1 P2 S3 O1 P3 Q2 O2 Q3 O3'
ORDER_COPY = 'S0 S1 S2 S3 P0 P1 O0 C0 P2 O1 C1 P3 O2 C2 O3 C3'
ORDER_LAST = 'S0 S1 S2 S3 P0 P1 O0 P2 O1 P3 O2 O3'


def _att_scores(b, q_scr, k_ref, p_scr, lane):
    r0 = b * SQ
    qs = jnp.concatenate(
        [q_scr[r0:r0 + SQ, h * DH:(h + 1) * DH] for h in range(HG)], axis=0)
    ks = k_ref[b].reshape(HG * SK, DH)
    st = lax.dot_general(ks, qs, (((1,), (1,)), ((), ())),
                         preferred_element_type=jnp.float32)
    c = st[0:SK]
    for h in range(1, HG):
        c = jnp.where(lane == h, st[h * SK:(h + 1) * SK], c)
    m = jnp.max(c, axis=0, keepdims=True)
    e = jnp.exp((c - m) * SCALE)
    l = jnp.sum(e, axis=0, keepdims=True)
    p = e * pl.reciprocal(l, approx=False)
    ptd = jnp.concatenate(
        [jnp.where(lane == h, p, 0.0) for h in range(HG)],
        axis=0).astype(jnp.bfloat16)
    p_scr[b] = ptd.T


def _att_pv(b, p_scr, v_ref, o_scr):
    r0 = b * SQ
    vs = v_ref[b].reshape(HG * SK, DH)
    o = jnp.dot(p_scr[b], vs,
                preferred_element_type=jnp.float32).astype(jnp.bfloat16)
    for h in range(HG):
        o_scr[r0:r0 + SQ, h * DH:(h + 1) * DH] = o[h * SQ:(h + 1) * SQ]


def _kernel(xa, ka, va, wqa, woa, xb, kb, vb, wqb, wob, out_hbm,
            x_buf, k_buf, v_buf, wq_buf, wo_buf, acc_ref, q_all, o_scr,
            p_scr, out_buf, x_sem, wq_sem, kv_sem, out_sem):
    st = pl.program_id(0)
    q_scr = q_all.at[0]
    q_tmp = q_all.at[1]

    def wq_copy(wq_hbm, gg, sl):
        return pltpu.make_async_copy(
            wq_hbm.at[:, pl.ds(pl.multiple_of(gg * HW, HW), HW)],
            wq_buf.at[sl], wq_sem.at[sl])

    def kvo_copies(refs, gg, sl):
        k_hbm, v_hbm, wo_hbm = refs
        return [
            pltpu.make_async_copy(k_hbm.at[:, pl.ds(gg * HG, HG)],
                                  k_buf.at[sl], kv_sem.at[sl, 0]),
            pltpu.make_async_copy(v_hbm.at[:, pl.ds(gg * HG, HG)],
                                  v_buf.at[sl], kv_sem.at[sl, 1]),
            pltpu.make_async_copy(
                wo_hbm.at[pl.ds(pl.multiple_of(gg * HW, HW), HW), :],
                wo_buf.at[sl], kv_sem.at[sl, 2]),
        ]

    def start_wq(ss):
        gg = ss % NG
        sl = ss % NSL

        @pl.when(ss < NG)
        def _():
            wq_copy(wqa, gg, sl).start()

        @pl.when(jnp.logical_and(ss >= NG, ss < NS))
        def _():
            wq_copy(wqb, gg, sl).start()

    def start_kvo(ss):
        gg = ss % NG
        sl = ss % NSL

        @pl.when(ss < NG)
        def _():
            for c in kvo_copies((ka, va, woa), gg, sl):
                c.start()

        @pl.when(jnp.logical_and(ss >= NG, ss < NS))
        def _():
            for c in kvo_copies((kb, vb, wob), gg, sl):
                c.start()

    def wait_kvo(ss):
        for c in kvo_copies((ka, va, woa), 0, ss % NSL):
            c.wait()

    def wait_wq(ss):
        wq_copy(wqa, 0, ss % NSL).wait()

    def xb_copy():
        return pltpu.make_async_copy(xb, x_buf.at[1], x_sem.at[0])

    def out_copy(blk, c=None):
        if c is None:
            return pltpu.make_async_copy(
                out_buf.at[blk], out_hbm.at[:, pl.ds(blk * D, D)],
                out_sem.at[0])
        return pltpu.make_async_copy(
            out_buf.at[blk, pl.ds(c * CR, CR)],
            out_hbm.at[pl.ds(c * CR, CR), pl.ds(blk * D, D)],
            out_sem.at[1 + c])

    def group(gi, last=False, copy_q=False):
        k_ref = k_buf.at[gi % NSL]
        v_ref = v_buf.at[gi % NSL]
        wo_ref = wo_buf.at[gi % NSL]
        lane = lax.broadcasted_iota(jnp.int32, (SK, HG * SQ), 1) // SQ
        not_first = (gi % NG) != 0
        o_ref = out_buf.at[gi // NG]

        def sph(c):
            for b in range(c * CB, (c + 1) * CB):
                _att_scores(b, q_scr, k_ref, p_scr, lane)

        def pvph(c):
            for b in range(c * CB, (c + 1) * CB):
                _att_pv(b, p_scr, v_ref, o_scr)

        def oproj(c):
            r = c * CR
            upd = jnp.dot(o_scr[r:r + CR, :], wo_ref[...],
                          preferred_element_type=jnp.float32)
            if isinstance(not_first, bool):
                new = acc_ref[r:r + CR, :] + upd if not_first else upd
            else:
                new = jnp.where(not_first, acc_ref[r:r + CR, :], 0.0) + upd
            if not last:
                acc_ref[r:r + CR, :] = new
            o_ref[r:r + CR, :] = new.astype(out_buf.dtype)
            if last:
                out_copy(1, c).start()

        def qchunk(c):
            r = c * CR
            x_ref = x_buf.at[(gi + 1) // NG]
            q = jnp.dot(x_ref[r:r + CR, :], wq_buf[(gi + 1) % NSL],
                        preferred_element_type=jnp.float32)
            q_scr[r:r + CR, :] = q.astype(jnp.bfloat16)

        order = ORDER_LAST if last else (ORDER_COPY if copy_q else ORDER)
        for tok in order.split():
            kind, idx = tok[0], int(tok[1:])
            if kind == 'S':
                sph(idx)
            elif kind == 'P':
                pvph(idx)
            elif kind == 'O':
                oproj(idx)
            elif kind == 'Q':
                qchunk(idx)
            else:
                q_scr[idx * CR:(idx + 1) * CR, :] = (
                    q_tmp[idx * CR:(idx + 1) * CR, :])

    @pl.when(st == 0)
    def _():
        def xc(c):
            return pltpu.make_async_copy(
                xa.at[pl.ds(c * XR, XR)], x_buf.at[0, pl.ds(c * XR, XR)],
                x_sem.at[1 + c])

        wq_copy(wqa, 0, 0).start()
        xc(0).start()
        wq_copy(wqa, 0, 0).wait()
        xc(0).wait()
        xc(1).start()
        start_wq(1)

        def qpiece(i, carry):
            @pl.when(i == 1)
            def _():
                xc(1).wait()
                start_kvo(0)

            @pl.when(i == 2)
            def _():
                wait_wq(1)
                start_kvo(1)
                start_wq(2)

            w = i // 2
            r0 = pl.multiple_of((i % 2) * XR, XR)
            for c in range(XR // CR):
                rows = pl.ds(pl.multiple_of(r0 + c * CR, CR), CR)
                q = jnp.dot(x_buf[0, rows, :], wq_buf[w],
                            preferred_element_type=jnp.float32)
                q_all[w, rows, :] = q.astype(jnp.bfloat16)
            return carry

        lax.fori_loop(0, 4, qpiece, 0)
        wait_kvo(0)
        start_kvo(2)
        start_wq(3)
        start_kvo(3)
        start_wq(4)
        group(0, copy_q=True)

    @pl.when(jnp.logical_or(st == 1, st == NSTEP - 2))
    def _():
        gi = jnp.where(st == 1, 1, NS - 2)
        wait_kvo(gi)
        wait_wq(gi + 1)
        group(gi)

    @pl.when(jnp.logical_and(st >= 2, st < NSTEP - 2))
    def _():
        g1 = 2 * st - 2

        @pl.when(st == NG // 2)
        def _():
            xb_copy().wait()

        wait_kvo(g1)
        wait_wq(g1 + 1)
        wait_kvo(g1 + 1)
        wait_wq(g1 + 2)
        start_kvo(g1 + 2)
        start_wq(g1 + 3)
        start_kvo(g1 + 3)
        start_wq(g1 + 4)

        @pl.when(st == 2)
        def _():
            xb_copy().start()

        group(g1)
        group(g1 + 1)

        @pl.when(st == NG // 2)
        def _():
            out_copy(0).start()

    @pl.when(st == NSTEP - 1)
    def _():
        wait_kvo(NS - 1)
        group(NS - 1, last=True)
        out_copy(0).wait()
        for c in range(NC):
            out_copy(1, c).wait()


@jax.jit
def pallas_concat_heads__mha_block_cached__mha_block_cached__near_ridge_kernel(
    A_x: jax.Array,
    A_k_cache: jax.Array,
    A_v_cache: jax.Array,
    A_wq: jax.Array,
    A_wo: jax.Array,
    B_x: jax.Array,
    B_k_cache: jax.Array,
    B_v_cache: jax.Array,
    B_wq: jax.Array,
    B_wo: jax.Array,
):
    xa = A_x.reshape(M, D)
    xb = B_x.reshape(M, D)
    bf = jnp.bfloat16
    out = pl.pallas_call(
        _kernel,
        grid=(NSTEP,),
        in_specs=[pl.BlockSpec(memory_space=pl.ANY)] * 10,
        out_specs=pl.BlockSpec(memory_space=pl.ANY),
        out_shape=jax.ShapeDtypeStruct((M, 2 * D), bf),
        scratch_shapes=[
            pltpu.VMEM((2, M, D), bf),
            pltpu.VMEM((NSL, B, HG, SK, DH), bf),
            pltpu.VMEM((NSL, B, HG, SK, DH), bf),
            pltpu.VMEM((NSL, D, HW), bf),
            pltpu.VMEM((NSL, HW, D), bf),
            pltpu.VMEM((M, D), jnp.float32),
            pltpu.VMEM((2, M, HW), bf),
            pltpu.VMEM((M, HW), bf),
            pltpu.VMEM((B, HG * SK, HG * SQ), bf),
            pltpu.VMEM((2, M, D), bf),
            pltpu.SemaphoreType.DMA((3,)),
            pltpu.SemaphoreType.DMA((NSL,)),
            pltpu.SemaphoreType.DMA((NSL, 3)),
            pltpu.SemaphoreType.DMA((1 + NC,)),
        ],
        compiler_params=pltpu.CompilerParams(
            dimension_semantics=("arbitrary",),
            vmem_limit_bytes=64 * 1024 * 1024,
            disable_bounds_checks=True,
        ),
    )(xa, A_k_cache, A_v_cache, A_wq, A_wo,
      xb, B_k_cache, B_v_cache, B_wq, B_wo)
    return out.reshape(B, SQ, 2 * D)
```
